```python
import os as _os
_os.environ.setdefault("JAX_PLATFORMS", "cpu")
import jax
import jax.numpy as jnp

def _softmax(x, axis=-1):
    return jax.nn.softmax(x, axis=axis)
def _gelu(x):
    return jax.nn.gelu(x, approximate=True)
def _silu(x):
    return jax.nn.silu(x)
def _sigmoid(x):
    return jax.nn.sigmoid(x)
def _layernorm(x, axis=-1, eps=1e-5):
    m = jnp.mean(x, axis=axis, keepdims=True)
    v = jnp.var(x, axis=axis, keepdims=True)
    return (x - m) / jnp.sqrt(v + eps)
def _scatter_add(tgt, idx, src, axis=0):
    return tgt.at[idx].add(src)
def _segment_sum(src, seg, n):
    return jax.ops.segment_sum(src, seg, n)
class _Rng:
    def __init__(self, key):
        self._k = key
    def _next(self):
        self._k, sub = jax.random.split(self._k)
        return sub
    def normal(self, shape):
        return jax.random.normal(self._next(), shape, dtype=jnp.bfloat16)
    def randint(self, lo, hi, shape):
        return jax.random.randint(self._next(), shape, lo, hi, dtype=jnp.int32)
    def uniform(self, shape, lo=0.0, hi=1.0):
        return jax.random.uniform(self._next(), shape, jnp.bfloat16, lo, hi)
    def permutation(self, n):
        return jax.random.permutation(self._next(), n)


kernel_name = 'concat_heads__mha_block_cached__mha_block_cached__near_ridge'

def setup_inputs():
    _rng = _Rng(jax.random.key(int.from_bytes(__import__("os").urandom(4), "little")))
    _w = (lambda a: (lambda t: t.astype(jnp.bfloat16) if jnp.issubdtype(t.dtype, jnp.floating) else t)(jnp.asarray(a)))
    def _A_setup():
        B, Sq, D = 16, 32, 1024
        H, Sk, Dh = 32, 32, 128
        return {
            "x": _w((lambda *s: _rng.normal(s) * 0.8)(B, Sq, D)),
            "k_cache": _w((lambda *s: _rng.normal(s) * 0.8)(B, H, Sk, Dh)),
            "v_cache": _w((lambda *s: _rng.normal(s) * 0.05)(B, H, Sk, Dh)),
            "wq": _w((lambda *s: _rng.normal(s) * 0.8)(D, H * Dh) * (D ** -0.5)),
            "wo": _w((lambda *s: _rng.normal(s) * 0.05)(H * Dh, D) * ((H * Dh) ** -0.5)),
        }
    _A_in = _A_setup()

    def _B_setup():
        B, Sq, D = 16, 32, 1024
        H, Sk, Dh = 32, 32, 128
        return {
            "x": _w((lambda *s: _rng.normal(s) * 0.8)(B, Sq, D)),
            "k_cache": _w((lambda *s: _rng.normal(s) * 0.8)(B, H, Sk, Dh)),
            "v_cache": _w((lambda *s: _rng.normal(s) * 0.05)(B, H, Sk, Dh)),
            "wq": _w((lambda *s: _rng.normal(s) * 0.8)(D, H * Dh) * (D ** -0.5)),
            "wo": _w((lambda *s: _rng.normal(s) * 0.05)(H * Dh, D) * ((H * Dh) ** -0.5)),
        }
    _B_in = _B_setup()

    return {
        "A_x": _A_in["x"],
        "A_k_cache": _A_in["k_cache"],
        "A_v_cache": _A_in["v_cache"],
        "A_wq": _A_in["wq"],
        "A_wo": _A_in["wo"],
        "B_x": _B_in["x"],
        "B_k_cache": _B_in["k_cache"],
        "B_v_cache": _B_in["v_cache"],
        "B_wq": _B_in["wq"],
        "B_wo": _B_in["wo"],
    }

def reference(A_x, A_k_cache, A_v_cache, A_wq, A_wo, B_x, B_k_cache, B_v_cache, B_wq, B_wo):
    def _A_ref(x, k_cache, v_cache, wq, wo):
        B, Sq, D = x.shape
        H, Dh = 32, 128
        q = (lambda x, *d: x.transpose(*d))((x @ wq).reshape(B, Sq, H, Dh), 0, 2, 1, 3)
        scores = jnp.einsum("bhqd,bhkd->bhqk", q, k_cache) * (Dh ** -0.5)
        p = _softmax(scores, axis=-1)
        o = jnp.einsum("bhqk,bhkd->bhqd", p, v_cache)
        return (lambda x, *d: x.transpose(*d))(o, 0, 2, 1, 3).reshape(B, Sq, H * Dh) @ wo

    def _B_ref(x, k_cache, v_cache, wq, wo):
        B, Sq, D = x.shape
        H, Dh = 32, 128
        q = (lambda x, *d: x.transpose(*d))((x @ wq).reshape(B, Sq, H, Dh), 0, 2, 1, 3)
        scores = jnp.einsum("bhqd,bhkd->bhqk", q, k_cache) * (Dh ** -0.5)
        p = _softmax(scores, axis=-1)
        o = jnp.einsum("bhqk,bhkd->bhqd", p, v_cache)
        return (lambda x, *d: x.transpose(*d))(o, 0, 2, 1, 3).reshape(B, Sq, H * Dh) @ wo

    a = _A_ref(A_x, A_k_cache, A_v_cache, A_wq, A_wo)
    b = _B_ref(B_x, B_k_cache, B_v_cache, B_wq, B_wo)
    return jnp.concatenate([a, b], axis=-1)
```

```python
import functools
import jax
import jax.numpy as jnp
from jax import lax
import jax.experimental.pallas as pl
import jax.experimental.pallas.tpu as pltpu

B, SQ, D = 16, 32, 1024
H, SK, DH = 32, 32, 128
M = B * SQ
MH = M // 2
BF = jnp.bfloat16
F32 = jnp.float32
U32 = jnp.uint32
LOG2E = 1.4426950408889634
G = 8
NG = H // G
NB = 4
TB = 2
T = (-1.5, -0.5, 0.5, 1.5)
PAIRS = [(i, j) for i in range(NB) for j in range(i + 1, NB)]
PRODS = [p for i, j in PAIRS for p in (("X", i, j), ("X", j, i), ("Y", i, j))] + [p for i in range(NB) for p in (("P", i, i), ("Q", i, i))]


def scores(q, k):
    lane_blk = lax.broadcasted_iota(jnp.int32, (SK, 128), 1) // SK
    st = []
    for g in range(4):
        s = lax.dot_general(k(g), q(g), (((1,), (1,)), ((), ())), preferred_element_type=F32)
        c = s[0:32]
        for j in range(1, 4):
            c = jnp.where(lane_blk == j, s[32 * j:32 * j + 32], c)
        st.append(c)
    return st


def softmax_t(st, tbf):
    out = []
    for c in st:
        m = jnp.max(c, axis=0, keepdims=True)
        e = jnp.exp2((c - m) * (DH ** -0.5 * LOG2E))
        l = jnp.sum(e, axis=0, keepdims=True)
        out.append(e * (1.0 / l))
    pt = jnp.concatenate(out, axis=0)
    return pt.astype(BF).T if tbf else pt.T.astype(BF)


def pv(p, v):
    pu = pltpu.bitcast(p, U32)
    cb = lax.broadcasted_iota(jnp.int32, (16, 128), 1) // 32
    o = [None] * 16
    for m_ in range(4):
        lhs = jnp.concatenate([jnp.where(cb == (c + m_) % 4, pu[16 * c:16 * c + 16], jnp.uint32(0)) for c in range(4)], axis=0)
        rhs = jnp.concatenate([v(4 * g + ((g - m_) % 4)) for g in range(4)], axis=0)
        r = jnp.dot(pltpu.bitcast(lhs, BF), rhs, preferred_element_type=F32)
        for c in range(4):
            o[4 * ((c + m_) % 4) + c] = r[32 * c:32 * c + 32]
    return jnp.concatenate(o[:8], axis=0), jnp.concatenate(o[8:], axis=0)


def scale(c, a):
    return a if c == 1.0 else (-a if c == -1.0 else c * a)


def axpy(c, a, y):
    return y + a if c == 1.0 else (y - a if c == -1.0 else y + c * a)


def parse(x):
    return [int(v) for v in str(x).lstrip("p").split("_")]


def build(nodma=False, flags="XLA_TPU_RESCHEDULE_DMA_DONES", nsteps=8, aoff=0.5, dbg=0, prods=None, pos=None, pos2=None,
          passes="QQOO", heads=None, tbf=1, merged=0, nsem=12, first=1, lim="p4_8_8_32", prods0=None, fence=2, ksplit=0, nmerged=1, splits=None, smode=0, maxq=56):
    FL = {}
    for f_ in (flags or "").split("+"):
        if f_: FL[f_] = True
    NS = nsteps
    NBR = 2 if NS > NG else 1
    porder = [PRODS[i] for i in parse(prods)] if prods is not None else list(PRODS)
    HEADS = parse(heads) if heads is not None else list(range(G))

    def proj_ops(kind, s, mode):
        if mode == 0:
            return [[(kind, s, c, p) for p in porder] for c in range(TB)]
        if mode == 1:
            order = [(i, j) for j in range(NB) for i in range(j)]
            grp = [[("X", i, j), ("X", j, i), ("Y", i, j)] for i, j in order] + [[("P", i, i), ("Q", i, i)] for i in range(NB)]
            ops = [(kind, s, c, p) for g_ in grp for c in range(TB) for p in g_]
            return [ops[:26], ops[26:]]
        if mode == 2:
            ops = [(kind, s, c, p) for p in porder for c in range(TB)]
            return [ops[:26], ops[26:]]

    def mode_of(kind, s):
        return 1 if (kind == "Q" and s < nmerged) else merged

    def col_of(kind, s, j, c):
        return j * TB + c if mode_of(kind, s) else c * NB + j

    prog = [o for l in proj_ops("Q", 0, mode_of("Q", 0)) for o in l]
    for s in range(NS):
        qs = proj_ops("Q", s + 1, mode_of("Q", s + 1)) if s + 1 < NS else []
        os_ = proj_ops("O", s - 1, merged) if s > 0 else []
        fill = []
        for ch in passes:
            lst = qs if ch == "Q" else os_
            if lst: fill += lst.pop(0)
        att = [("S", s, HEADS[0])]
        for a in range(G):
            if a + 1 < G: att.append(("S", s, HEADS[a + 1]))
            att.append(("V", s, HEADS[a]))
        pp = pos if len(fill) > 60 else pos2
        pp = [int((k + aoff) / len(att) * len(fill) + 0.5) for k in range(len(att))] if pp is None else parse(pp)
        for n_ in range(len(fill) + 1):
            while att and pp[0] <= n_:
                pp.pop(0); prog.append(att.pop(0))
            if n_ < len(fill): prog.append(fill[n_])
        assert not att
    prog += [o for l in proj_ops("O", NS - 1, merged) for o in l]

    def blocks_of(p):
        kind, i, j = p
        if kind == "X": return [(i, j)]
        if kind == "Y": return [(i, j), (j, i)]
        if kind == "P": return [(i, m) for m in range(NB)]
        return [(m, i) for m in range(NB)]

    def items_of(op):
        if op[0] == "S": return [(("k", op[1], op[2]), 2)]
        if op[0] == "V": return [(("v", op[1], op[2]), 2)]
        kind, s, c, p = op
        its = []
        if kind == "Q":
            its += [(("x", s // NG, i), 4) for i in sorted({p[1], p[2]})]
        for i, j in blocks_of(p):
            w = "wq" if kind == "Q" else "wo"
            its.append(((w, s, i, j * TB, TB), 2) if mode_of(kind, s) else ((w, s, i, c * NB, NB), 4))
        return its

    L = parse(lim)
    groups, seen, cum, gsz = [], set(), 0, 0
    wait_at = {}
    for n_, op in enumerate(prog):
        for key, sz in items_of(op):
            if key in seen: continue
            seen.add(key)
            limit = L[0] if cum < 48 else (L[1] if cum < 112 else (L[2] if cum < 208 else L[3]))
            if not groups or gsz >= limit:
                groups.append([]); gsz = 0
                wait_at.setdefault(n_, []).append(len(groups) - 1)
            groups[-1].append(key); gsz += sz; cum += sz

    def merge(keys):
        out = []
        for key in sorted(keys):
            if len(key) == 5 and out and len(out[-1][0]) == 5 and out[-1][0][:3] == key[:3] and out[-1][0][3] + out[-1][0][4] == key[3]:
                out[-1][0] = key[:3] + (out[-1][0][3], out[-1][0][4] + key[4])
            else:
                out.append([key, 1])
        res = []
        for key, _ in sorted(out, key=lambda z: (z[0][:2], z[0][3:], z[0][2])):
            if res and res[-1][0][:2] == key[:2] and res[-1][0][3:] == key[3:] and res[-1][0][2] + res[-1][1] == key[2]:
                res[-1][1] += 1
            else:
                res.append([key, 1])
        rank = {k[:3]: n for n, k in reversed(list(enumerate(keys)))}
        return sorted(res, key=lambda z: rank[z[0][:3]])
    groups = [merge(g_) for g_ in groups]

    def kernel(ax, ak, av, awq, awo, bx, bk, bv, bwq, bwo, out, x_v, k_v, v_v, wq_v, wo_v, o_v, fence_v, sem, sem_o, sem_r):
        xs, ks, vs, wqs, wos = (ax, bx), (ak, bk), (av, bv), (awq, bwq), (awo, bwo)

        def copies(gi):
            sm = sem.at[gi % nsem]
            cs = []
            for key, n in groups[gi]:
                kind = key[0]
                if kind == "x":
                    _, br, i = key
                    cols = pl.ds(i * TB * 128, n * TB * 128)
                    cs.append(pltpu.make_async_copy(xs[br].at[:, cols], x_v.at[br, :, cols], sm))
                    continue
                s = key[1]
                br, g = divmod(s, NG)
                if kind in ("k", "v"):
                    src, dst = (ks[br], k_v) if kind == "k" else (vs[br], v_v)
                    cs.append(pltpu.make_async_copy(src.at[:, pl.ds(g * G + key[2], n)], dst.at[s, :, pl.ds(key[2], n)], sm))
                    continue
                _, _, i, c0, nc = key
                for par in range(2):
                    if kind == "wq":
                        src = wqs[br].at[pl.ds(i * 16, 16 * n), par, pl.ds(g * G + c0, nc)]
                    else:
                        src = wos[br].at[pl.ds(g * 64 + i * 16, 16 * n), par, pl.ds(c0, nc)]
                    dst = (wq_v if kind == "wq" else wo_v).at[s, pl.ds(i * 16, 16 * n), pl.ds(c0, nc), pl.ds(8 * par, 8)]
                    cs.append(pltpu.make_async_copy(src, dst, sm))
            return cs

        def start(gi):
            if nodma or gi >= len(groups): return
            for c in copies(gi): c.start()

        def wait(gi):
            if nodma or dbg == 1: return
            for c in copies(gi): c.wait()

        f = lambda a: a.astype(F32)
        bf = lambda a: a.astype(BF)

        def a_pair(a1, a2, i, j):
            tau = T[j] - T[i]
            s_ = axpy(T[i], a1(i), a2(i)) + axpy(T[j], a1(j), a2(j))
            return {("Y", i, j): bf(s_), ("X", i, j): bf(axpy(tau, a1(i), s_)), ("X", j, i): bf(axpy(-tau, a1(j), s_))}

        def a_diag(a1, a2, i):
            return {("P", i, i): bf(a1(i)), ("Q", i, i): bf(axpy(T[i], a1(i), a2(i)))}

        xa, oa, of, qv, acc = {}, {}, {}, {}, {}

        def x_operand(br, p):
            kind, i, j = p
            if (br, p) not in xa:
                a1 = lambda m: f(x_v[br, 0:MH, pl.ds(m * TB * 128, TB * 128)])
                a2 = lambda m: f(x_v[br, MH:M, pl.ds(m * TB * 128, TB * 128)])
                d = a_diag(a1, a2, i) if i == j else a_pair(a1, a2, min(i, j), max(i, j))
                for pp_, val in d.items(): xa[(br, pp_)] = val
            return xa[(br, p)]

        def b_operand(w_v, s, p, c, cc=None):
            kind, i, j = p
            wk = "Q" if w_v is wq_v else "O"

            def blk(r, cb):
                if cc is not None:
                    u = w_v.bitcast(U32)[s, pl.ds(r * 16 + cc * 8, 8), col_of(wk, s, cb, c)]
                    return pltpu.bitcast(u.reshape(64, 128), BF)
                col = col_of(wk, s, cb, c)
                rows = pl.ds(r * 16, 16)
                if fence != 2 or kind == "X":
                    u = w_v.bitcast(U32)[s, rows, col]
                elif kind == "Y":
                    u = w_v.bitcast(U32).at[s][rows, col]
                elif kind == "P":
                    u = w_v.bitcast(U32).at[s, rows][:, col]
                else:
                    u = w_v.bitcast(U32).at[:, rows][s, :, col]
                return pltpu.bitcast(u.reshape(128, 128), BF)
            if kind == "X":
                return blk(i, j)
            if kind == "Y":
                return bf(f(blk(j, i)) - f(blk(i, j)))
            r = f(blk(i, i))
            for m in range(NB):
                if m != i:
                    r = r - f(blk(i, m) if kind == "P" else blk(m, i))
            return bf(r)

        state = {}

        def product(kind, s, c, p):
            br, g = divmod(s, NG)
            last = g == NG - 1 or s == NS - 1
            st = state.setdefault((kind, s, c), {"cnt": [0] * NB})
            pk, i, j = p
            if fence == 1: fence_v[...] = jnp.zeros((8, 128), F32)
            if kind == "Q":
                r = jnp.dot(x_operand(br, p), b_operand(wq_v, s, p, c), preferred_element_type=F32)
            else:
                if ksplit:
                    r = None
                    for cc in range(TB):
                        rr = jnp.dot(oa[(s, p, cc)], b_operand(wo_v, s, p, c, cc), preferred_element_type=F32)
                        r = rr if r is None else r + rr
                else:
                    r = jnp.dot(oa[(s, p)], b_operand(wo_v, s, p, c), preferred_element_type=F32)

            def add(key, val):
                prev = st.get(key)
                if prev is None and kind == "O" and g > 0: prev = acc[(c,) + key]
                st[key] = val if prev is None else prev + val

            if pk == "P":
                add(("G", i), r); touched = [i]
            elif pk == "Q":
                add(("D", i), r); touched = [i]
            else:
                a, b = min(i, j), max(i, j)
                if pk == "X": add(("D", j), r)
                neg = pk == "X" and i > j
                key = ("W", a, b)
                if key not in st:
                    st[key] = (r, neg, 1)
                else:
                    w, wneg, k = st[key]
                    if wneg and not neg: w, wneg = r - w, False
                    elif wneg == neg: w = w + r
                    else: w = w - r
                    st[key] = (w, wneg, k + 1)
                    if k + 1 == 3:
                        w = scale(1.0 / (T[b] - T[a]), w)
                        add(("G", a), w); add(("G", b), w)
                touched = [a, b]
            for m in touched:
                st["cnt"][m] += 1
                if st["cnt"][m] < 2 + 3 * (NB - 1): continue
                gam, dele = st[("G", m)], st[("D", m)]
                col = col_of(kind, s, m, c)
                if kind == "Q":
                    c2 = axpy(-T[m], gam, dele)
                    qv[(s, col)] = [bf(gam[0:128]), bf(gam[128:256]), bf(c2[0:128]), bf(c2[128:256])]
                elif not last:
                    acc[(c, "G", m)], acc[(c, "D", m)] = gam, dele
                else:
                    pending_out.append((br, col, gam, axpy(-T[m], gam, dele)))

        def ocopy(br, j):
            return pltpu.make_async_copy(o_v.at[br, j], out.at[:, pl.ds(br * D + j * 128, 128)], sem_o)

        ps = {}
        pending_out = []

        def S(s, h):
            q = qv.pop((s, h))
            k = lambda g: pltpu.bitcast(k_v.bitcast(U32)[s, 4 * g:4 * g + 4, h].reshape(64, DH), BF)
            ps[(s, h)] = softmax_t(scores(lambda g: q[g], k), tbf)

        def PV(s, h):
            of[(s, h)] = pv(ps.pop((s, h)), lambda b: pltpu.bitcast(v_v.bitcast(U32)[s, b, h], BF))
            i, c = divmod(h, TB)
            if ksplit:
                a1 = lambda m: of[(s, m * TB + c)][0]
                a2 = lambda m: of[(s, m * TB + c)][1]
                have = lambda m: (s, m * TB + c) in of
            else:
                a1 = lambda m: jnp.concatenate([of[(s, m * TB + cc)][0] for cc in range(TB)], axis=1)
                a2 = lambda m: jnp.concatenate([of[(s, m * TB + cc)][1] for cc in range(TB)], axis=1)
                have = lambda m: all((s, m * TB + cc) in of for cc in range(TB))
                if not have(i): return
            d = a_diag(a1, a2, i)
            for m in range(NB):
                if m != i and have(m):
                    d.update(a_pair(a1, a2, min(i, m), max(i, m)))
            for pp_, val in d.items():
                oa[(s, pp_, c) if ksplit else (s, pp_)] = val

        ndesc = [sum(2 if len(k) == 5 else 1 for k, _ in g_) for g_ in groups]
        nxt = [0]

        def top_up(done):
            while nxt[0] < len(groups) and nxt[0] - done < nsem and sum(ndesc[done:nxt[0] + 1]) <= maxq:
                start(nxt[0]); nxt[0] += 1

        top_up(0)
        cuts = [] if splits is None else [int(len(prog) * v / 100) for v in parse(splits)]
        for n_, op in enumerate(prog):
            if n_ in cuts:
                if smode == 0:
                    pl.semaphore_signal(sem_r, 1)
                    pl.semaphore_wait(sem_r, 1)
                elif smode == 1:
                    pl.delay(1)
                elif smode == 2:
                    def body(i_, c_):
                        fence_v[...] = jnp.zeros((8, 128), F32)
                        return c_
                    lax.fori_loop(0, pl.semaphore_read(sem_r), body, 0)
            for gi in wait_at.get(n_, []):
                wait(gi)
                top_up(gi + 1)
            if dbg == 2: continue
            if op[0] == "S": S(op[1], op[2])
            elif op[0] == "V": PV(op[1], op[2])
            else: product(*op)
            if nxt[0] >= len(groups):
                while pending_out:
                    br, col, c1, c2 = pending_out.pop(0)
                    o_v[br, col, 0:MH] = bf(c1)
                    o_v[br, col, MH:M] = bf(c2)
                    ocopy(br, col).start()
        if dbg == 2: return
        if dbg == 1:
            for gi in range(len(groups)):
                for c in copies(gi): c.wait()
        for br in range(NBR):
            for j in range(G): ocopy(br, j).wait()

    @jax.jit
    def fn(A_x, A_k, A_v, A_wq, A_wo, B_x, B_k, B_v, B_wq, B_wo):
        any_spec = pl.BlockSpec(memory_space=pl.ANY)
        tiles = lambda w: w.reshape(w.shape[0] // 16, 2, 8, w.shape[1] // 128, 128).transpose(0, 1, 3, 2, 4)
        out = pl.pallas_call(
            kernel,
            out_shape=jax.ShapeDtypeStruct((M, 2 * D), BF),
            in_specs=[any_spec] * 10,
            out_specs=any_spec,
            scratch_shapes=[
                pltpu.VMEM((2, M, D), BF),
                pltpu.VMEM((NS, B, G, SK, DH), BF),
                pltpu.VMEM((NS, B, G, SK, DH), BF),
                pltpu.VMEM((NS, 64, G, 16, 128), BF),
                pltpu.VMEM((NS, 64, G, 16, 128), BF),
                pltpu.VMEM((2, G, M, 128), BF),
                pltpu.VMEM((8, 128), F32),
                pltpu.SemaphoreType.DMA((nsem,)),
                pltpu.SemaphoreType.DMA(()),
                pltpu.SemaphoreType.REGULAR,
            ],
            compiler_params=pltpu.CompilerParams(vmem_limit_bytes=120 * 1024 * 1024, flags=FL or None),
        )(A_x.reshape(M, D), A_k, A_v, tiles(A_wq), tiles(A_wo), B_x.reshape(M, D), B_k, B_v, tiles(B_wq), tiles(B_wo))
        return out.reshape(B, SQ, 2 * D)
    return fn


@jax.jit
def pallas_concat_heads__mha_block_cached__mha_block_cached__near_ridge_kernel(
        A_x, A_k_cache, A_v_cache, A_wq, A_wo, B_x, B_k_cache, B_v_cache, B_wq, B_wo):
    return build()(A_x, A_k_cache, A_v_cache, A_wq, A_wo, B_x, B_k_cache, B_v_cache, B_wq, B_wo)
```

```python
import jax
import jax.numpy as jnp
from jax import lax
import jax.experimental.pallas as pl
import jax.experimental.pallas.tpu as pltpu

B, SQ, D = 16, 32, 1024
H, SK, DH = 32, 32, 128
M = B * SQ
MH = M // 2
G = 8
NS = H // G
NB = 4
TB = 2
KB = TB * 128
BF16, F32, U32 = jnp.bfloat16, jnp.float32, jnp.uint32
LOG2E = 1.4426950408889634

NODES = (-1.5, -0.5, 0.5, 1.5)

_ORDER = (
    """
    q0X01 q1X01 q0X10 q1Y01 q1X10 q0Y01 q0X10+1 q1X01+1 q1X10+1 q0X01+1 q0Y01+1 q1Y01+1 q0X01+2
    q1X10+2 q0Y01+2 q1Y01+2 q1X01+2 q0X01+3 q0X10+2 q1X01+3 q0X10+3 q1X10+3 q1Y01+3 q1X02 q0X02
    q0Y01+3 q0X20 q1X20 q1X12 q1Y02 q0X12 q0Y02 q0X21 q0Y12 q1X21 q0X03 q1X03 q1Y12 q0Y03 q0X30
    q1X13 q1Y03 q0X13 q1X31 q0P0 q1X30 q1P0 q0X31 q0Y13 q0Q0 q1X23 q0X23 q1Y13 q0X32 q1Q0 q1X32
    q0P1 q0Q1 q0P2 q1P2 q1P1 q0Q2 q1Q2 q0Y23 q1Y23 q1Q1 q0Q3 q1P3 q1Q3 q0P3
    """,
    """
    q0P0 q0X02 q0X03 S0 q0Y02 S1 q0X20 q0Y03 S2 q0X30 q0P1 V0 q0Y12 q0X12 q0Q0 q0Q1 V1 q0X21 S3
    q0X31 q0Y13 q0X13 q0P2 q0X23 V2 q0X32 q0Y23 q0P3 q0Q3 q0Q2 S4 q1X02 V3 q1P0 q1X20 q1Q0 V4
    q1X30 q1X03 q1Y03 S5 q1Y02 S6 q1P1 q1Y12 q1X21 q1Q1 V5 q1X12 q1X13 q1Y13 S7 q1X31 q1P2 q1X23
    q1X32 V6 q1Q2 q1Y23 q1P3 V7 q1Q3
    """,
    """
    q0X03 q0Q0 S0 q0P0 q0X02 q0X20 q0X30 q0Y02 S1 q0Y03 q0X12 q0P1 q0X21 V0 q0Y12 q0X13 q0Q1
    q0X31 q0Y13 q0X23 q0X32 q0Y23 q0P3 q0Q2 q0Q3 S2 V1 q1X30 q0P2 q1X20 q1X02 q1Y02 q1P0 q1X03
    V2 S3 q1Y03 q1X12 q1X21 q1Q0 q1Q1 q1P1 q1X13 q1Y12 q1X31 q1Q2 q1P2 q1X32 q1X23 o0X02 q1Y13
    q1Y23 S4 o0X10 q1Q3 o0X01 o0X30 V3 o0Y01 q1P3 o0P0 S5 o0Q0 o0X13 o0Y02 o0X20 o0X03 o0Y03
    o0X12 o0X21 o0P1 o0Y12 o0Q1 o0X31 o0Y13 o0P2 V4 o0X23 S6 o0X32 o0Y23 o0P3 o0Q2 o1Y01 o1X20
    o1X01 o1X10 o0Q3 o1P0 o1Y02 V5 o1X02 o1Q0 o1X03 o1X30 o1Y03 S7 o1P1 o1X12 o1Y12 o1Q1 o1X21
    V6 o1X13 o1X32 o1X31 o1Y13 o1P2 o1X23 o1Y23 o1Q2 o1P3 o1Q3 V7
    """,
    """
    q0X20 q0P0 q0P1 q0X02 q0Y02 q0Q0 S1 q0P2 S0 q0X03 q0X30 q0Y03 q0X12 q0Y12 q0X13 q0X21 q0Q1
    q0Y13 q0X31 q0X23 S2 q0X32 q0Y23 q0Q2 V0 q0P3 q1X02 q0Q3 q1P1 q1P0 q1X12 V1 q1X20 q1Q0 q1Y02
    q1X03 q1X30 q1X21 q1Y03 q1Y12 q1Q1 S3 V2 q1X13 S4 q1P2 q1X31 q1X23 q1Y13 q1Q2 q1P3 q1X32
    q1Y23 q1Q3 o0X01 o0X10 o0Y01 o0P0 o0X02 V3 V4 o0X20 o0X03 o0Y02 o0Q0 o0X30 o0Q1 o0X21 o0P1
    o0X12 o0Y12 o0Y03 o0X13 o0Y13 o0X31 o0X23 o0P2 S5 o0Y23 o0X32 S6 o0Q2 o0P3 o0Q3 o1X01 o1X10
    V5 o1Y01 o1X02 o1P0 o1X20 o1Q0 o1X03 o1X30 o1Y02 S7 o1Y03 o1P1 o1X32 o1X12 o1Q1 o1Y12 V6
    o1X13 o1X31 o1Y13 o1P2 o1X23 o1X21 o1Y23 V7 o1P3 o1Q3 o1Q2
    """,
    """
    o0X01 o0X10 S0 o0P0 o0Y01 o0X02 S1 o0X20 V0 o0Y02 o0Q0 o0X30 o0X03 o0Y03 S2 o0X21 o0X12 S4
    o0Y12 o0X13 o0Y13 o0X31 o0Q1 S3 o0P2 o0P1 o0X23 V2 o0Q2 V1 o0Y23 V3 o0Q3 o1X01 o1X30 o1Y01
    o0P3 o1X02 o1Q0 o1X20 o0X32 o1Y02 o1P0 S5 o1X10 o1X03 V4 S6 o1Y03 o1P1 o1X12 o1Y12 V5 o1X13
    o1X31 o1Q1 o1X21 S7 o1X23 V6 o1P2 o1Y13 o1X32 o1Y23 o1Q2 V7 o1Q3 o1P3
    """,
    """
    o0X01 o0Y01 o0X02 o0P0 o0Y12 o0X03 o0Y03 o0X10 o0Q0 o0Y13 o0X21 o0X32 o0X31 o0Q2 o0X12 o0X30
    o0P1 o0X13 o0X23 o0Q3 o0Y23 o1X01 o0X20 o0Q1 o1X10 o0P3 o0Y02 o1P0 o1Y01 o1X13 o1X02 o0P2
    o1X20 o1Y02 o1P1 o1Q0 o1Y13 o1X31 o1X30 o1X21 o1Y03 o1X03 o1Y23 o1Y12 o1X12 o1X32 o1X23 o1Q1
    o1P2 o1Q2 o1P3 o1Q3
    """,
)

_FIRST_GROUPS = (8, 4, 4, 4, 2, 4, 4, 2, 4, 4, 4, 2, 3, 4, 4)
_GROUP_SIZE = ((112, 6), (208, 8), (320, 16), (400, 32))
_NSEM = 16
_MAX_COPIES = 60
_MAX_AHEAD = 250
_EARLY_WAIT = (208, 10)


def _program():
    ops = []
    for phase, text in enumerate(_ORDER):
        for word in text.split():
            if word[0] in "SV":
                ops.append((word[0], phase - 1, int(word[1])))
            else:
                word, _, ahead = word.partition("+")
                group = phase + int(ahead or 0) if word[0] == "q" else phase - 2
                ops.append((word[0], group, int(word[1]), (word[2], int(word[3]), int(word[-1]))))
    return ops


def _tile(proj, s, block, c):
    return block * TB + c if (proj, s) == ("q", 0) else c * NB + block


def _weight_blocks(prod):
    name, i, j = prod
    if name == "X":
        return [(i, j)]
    if name == "Y":
        return [(i, j), (j, i)]
    return [(i, m) if name == "P" else (m, i) for m in range(NB)]


def _inputs_of(op, exact):
    if op[0] in "SV":
        return [(("k" if op[0] == "S" else "v", op[1], op[2]), 2)]
    proj, s, c, prod = op
    pieces = []
    if proj == "q":
        pieces += [(("x", 0, i), 4) for i in sorted({prod[1], prod[2]})]
    for i, j in _weight_blocks(prod):
        if (proj, s) == ("q", 0):
            pieces.append((("wq", s, i, j * TB, TB), TB))
        else:
            rows = [i] if exact else range(NB)
            pieces += [(("w" + proj, s, r, c * NB + j, 1), 1) for r in rows]
    return pieces


def _coalesce(keys):
    wide = []
    for key in sorted(keys):
        last = wide[-1] if wide else ()
        if len(key) == 5 and len(last) == 5 and last[:3] == key[:3] and last[3] + last[4] == key[3]:
            wide[-1] = key[:3] + (last[3], last[4] + key[4])
        else:
            wide.append(key)
    tall = []
    for key in sorted(wide, key=lambda k: (k[:2], k[3:], k[2])):
        if tall and tall[-1][0][:2] == key[:2] and tall[-1][0][3:] == key[3:] \
                and tall[-1][0][2] + tall[-1][1] == key[2]:
            tall[-1][1] += 1
        else:
            tall.append([key, 1])
    rank = {k[:3]: n for n, k in reversed(list(enumerate(keys)))}
    return sorted(tall, key=lambda z: rank[z[0][:3]])


def _copy_plan(ops):
    groups, sizes, seen, planned = [], [], set(), 0
    wait_at, last_use, x_done = {}, {}, set()
    for n, op in enumerate(ops):
        starting = n < len(_ORDER[0].split())
        for key, size in _inputs_of(op, starting):
            if key[0] != "x" or op[3][1:] not in x_done:
                last_use[key] = n
            if key in seen:
                continue
            seen.add(key)
            limit = next(size_ for until, size_ in _GROUP_SIZE if planned < until)
            if 0 < len(groups) <= len(_FIRST_GROUPS):
                limit = _FIRST_GROUPS[len(groups) - 1]
            inside_column = not starting and len(key) == 5 and key[4] == 1 and key[2] > 0
            if not groups or (sizes[-1] >= limit and not inside_column):
                groups.append([])
                sizes.append(0)
                early = _EARLY_WAIT[1] if planned >= _EARLY_WAIT[0] else 0
                wait_at.setdefault(max(0, n - early), []).append(len(groups) - 1)
            groups[-1].append(key)
            sizes[-1] += size
            planned += size
        if op[0] == "q":
            x_done.update({op[3][1:], op[3][:0:-1]})
    dead_after = [max(last_use[key] for key in group) for group in groups]
    groups = [_coalesce(group) for group in groups]
    copies = [sum(key[4] if len(key) == 5 else 1 for key, _ in group) for group in groups]
    ng = len(groups)
    ahead, start_at = [], {}

    def can_start(u, waited, now):
        if any(w % ng % _NSEM == u % ng % _NSEM for w in range(waited, u)):
            return False
        flight = range(waited, u + 1)
        twice = lambda w: w < ng and w not in ahead and now >= 0
        if sum(copies[w % ng] * (2 if twice(w) else 1) for w in flight) > _MAX_COPIES:
            return False
        if sum(sizes[w % ng] for w in flight) > _MAX_AHEAD:
            return False
        return u < ng or (u - ng < waited and dead_after[u - ng] < now)

    nxt = 0
    while nxt < ng and can_start(nxt, 0, -1):
        ahead.append(nxt)
        nxt += 1
    waited = 0
    for n in range(len(ops)):
        waited += len(wait_at.get(n, []))
        while nxt < ng + len(ahead) and can_start(nxt, waited, n):
            start_at.setdefault(n, []).append(nxt)
            nxt += 1
    assert nxt == ng + len(ahead)
    return groups, wait_at, start_at, ahead


def _axpy(c, a, y):
    return y + a if c == 1.0 else (y - a if c == -1.0 else y + c * a)


def _probabilities(q, k):
    lane_block = lax.broadcasted_iota(jnp.int32, (SK, 128), 1) // SQ
    probs = []
    for g in range(4):
        s = lax.dot_general(k(g), q[g], (((1,), (1,)), ((), ())), preferred_element_type=F32)
        low = jnp.where(lane_block == 1, s[SK:2 * SK], s[0:SK])
        high = jnp.where(lane_block == 3, s[3 * SK:4 * SK], s[2 * SK:3 * SK])
        s = jnp.where(lane_block >= 2, high, low) * (DH ** -0.5 * LOG2E)
        e = jnp.exp2(s - jnp.max(s, axis=0, keepdims=True))
        probs.append(e * (1.0 / jnp.sum(e, axis=0, keepdims=True)))
    return jnp.concatenate(probs, axis=0).T.astype(BF16)


def _weighted_values(p, v):
    packed = pltpu.bitcast(p, U32)
    lane_block = lax.broadcasted_iota(jnp.int32, (SQ // 2, 128), 1) // SK
    out = [None] * B
    for m in range(4):
        lhs = jnp.concatenate(
            [jnp.where(lane_block == (c + m) % 4, packed[16 * c:16 * c + 16], jnp.uint32(0))
             for c in range(4)], axis=0)
        rhs = jnp.concatenate([v(4 * g + (g - m) % 4) for g in range(4)], axis=0)
        r = jnp.dot(pltpu.bitcast(lhs, BF16), rhs, preferred_element_type=F32)
        for c in range(4):
            out[4 * ((c + m) % 4) + c] = r[SQ * c:SQ * (c + 1)]
    return jnp.concatenate(out[:B // 2], axis=0), jnp.concatenate(out[B // 2:], axis=0)


def _left_pair(a1, a2, i, j):
    tau = NODES[j] - NODES[i]
    s = _axpy(NODES[i], a1(i), a2(i)) + _axpy(NODES[j], a1(j), a2(j))
    return {("Y", i, j): s.astype(BF16),
            ("X", i, j): _axpy(tau, a1(i), s).astype(BF16),
            ("X", j, i): _axpy(-tau, a1(j), s).astype(BF16)}


def _left_single(a1, a2, i):
    return {("P", i, i): a1(i).astype(BF16),
            ("Q", i, i): _axpy(NODES[i], a1(i), a2(i)).astype(BF16)}


def _both_blocks(ax, ak, av, awq, awo, bx, bk, bv, bwq, bwo, out,
                 x_v, k_v, v_v, wq_v, wo_v, o_v, fence_v, in_sem, out_sem):
    xs, ks, vs, wqs, wos = (ax, bx), (ak, bk), (av, bv), (awq, bwq), (awo, bwo)
    ops = _program()
    groups, wait_at, start_at, ahead = _copy_plan(ops)
    ng = len(groups)

    def copies(gi, src, on=1):
        sem = in_sem.at[gi % _NSEM]
        for key, n in groups[gi]:
            kind, s = key[0], key[1]
            if kind == "x":
                cols = pl.ds(key[2] * KB, n * KB)
                lead = pl.ds(0, B * on)
                dst = x_v.at[lead, :, cols]
                yield pltpu.make_async_copy(
                    dst if src is None else xs[src].at[lead, :, cols], dst, sem)
            elif kind in ("k", "v"):
                hbm, vmem = (ks, k_v) if kind == "k" else (vs, v_v)
                lead = pl.ds(0, B * on)
                dst = vmem[s].at[lead, pl.ds(key[2], n)]
                yield pltpu.make_async_copy(
                    dst if src is None else hbm[src].at[lead, pl.ds(s * G + key[2], n)], dst, sem)
            else:
                _, _, i, c0, nc = key
                w_v = (wq_v if kind == "wq" else wo_v)[s]
                if src is None:
                    dst = w_v.at[pl.ds(c0, nc), pl.ds(i * KB, KB * n)]
                    yield pltpu.make_async_copy(dst, dst, sem)
                    continue
                rows = KB * n if isinstance(on, int) else pl.multiple_of(KB * n * on, KB)
                for c in range(c0, c0 + nc):
                    if kind == "wq":
                        piece = wqs[src].at[pl.ds(i * KB, rows), pl.ds((s * G + c) * 128, 128)]
                    else:
                        piece = wos[src].at[pl.ds(s * G * DH + i * KB, rows), pl.ds(c * 128, 128)]
                    yield pltpu.make_async_copy(piece, w_v.at[c, pl.ds(i * KB, rows)], sem)

    def right_operand(proj, s, prod, c):
        w_v = (wq_v if proj == "q" else wo_v)[s]
        name, i, j = prod
        block = lambda r, col: w_v[_tile(proj, s, col, c), pl.ds(r * KB, KB)]
        if name == "X":
            return block(i, j)
        if name == "Y":
            return (block(j, i).astype(F32) - block(i, j).astype(F32)).astype(BF16)
        w = block(i, i).astype(F32)
        for m in range(NB):
            if m != i:
                w = w - (block(i, m) if name == "P" else block(m, i)).astype(F32)
        return w.astype(BF16)

    def attention_block(blk, trips):
        x_left, o_left, heads, queries, probs = {}, {}, {}, {}, {}
        carried, partial, results = {}, {}, []

        def x_operand(prod):
            _, i, j = prod
            if prod not in x_left:
                a1 = lambda m: x_v[0:B // 2, :, pl.ds(m * KB, KB)].reshape(MH, KB).astype(F32)
                a2 = lambda m: x_v[B // 2:B, :, pl.ds(m * KB, KB)].reshape(MH, KB).astype(F32)
                x_left.update(_left_single(a1, a2, i) if i == j
                              else _left_pair(a1, a2, min(i, j), max(i, j)))
            return x_left[prod]

        def product(proj, s, c, prod):
            last = s == NS - 1
            sums = partial.setdefault((proj, s, c), {"missing": {m: [NB, NB] for m in range(NB)}})
            name, i, j = prod
            fence_v[...] = jnp.zeros((8, 128), F32)
            left = x_operand(prod) if proj == "q" else o_left[(s, prod)]
            r = jnp.dot(left, right_operand(proj, s, prod, c), preferred_element_type=F32)

            def accumulate(half, m, value):
                before = sums.get((half, m))
                if before is None and proj == "o" and s > 0:
                    before = carried[(c, half, m)]
                sums[(half, m)] = value if before is None else before + value
                missing = sums["missing"][m]
                missing[half] -= 1
                tile = _tile(proj, s, m, c)
                if proj == "o" and last and half == 0 and missing[0] == 0:
                    results.append((tile, 0, sums[(0, m)]))
                if missing != [0, 0]:
                    return
                first, rest = sums[(0, m)], sums[(1, m)]
                if proj == "q":
                    second = _axpy(-NODES[m], first, rest)
                    queries[(s, tile)] = [first[0:128].astype(BF16), first[128:256].astype(BF16),
                                          second[0:128].astype(BF16), second[128:256].astype(BF16)]
                elif not last:
                    carried[(c, 0, m)], carried[(c, 1, m)] = first, rest
                else:
                    results.append((tile, 1, _axpy(-NODES[m], first, rest)))

            if name == "P":
                accumulate(0, i, r)
            elif name == "Q":
                accumulate(1, i, r)
            else:
                lo, hi = min(i, j), max(i, j)
                if name == "X":
                    accumulate(1, j, r)
                minus = name == "X" and i > j
                if (lo, hi, "Z") not in sums:
                    sums[(lo, hi, "Z")] = (r, minus, 1)
                    return
                z, z_minus, terms = sums[(lo, hi, "Z")]
                if z_minus and not minus:
                    z, z_minus = r - z, False
                elif z_minus == minus:
                    z = z + r
                else:
                    z = z - r
                sums[(lo, hi, "Z")] = (z, z_minus, terms + 1)
                if terms + 1 == 3:
                    scale = 1.0 / (NODES[hi] - NODES[lo])
                    z = z if scale == 1.0 else scale * z
                    accumulate(0, lo, z)
                    accumulate(0, hi, z)

        def scores(s, h):
            keys = lambda g: k_v[s][4 * g:4 * g + 4, h].reshape(4 * SK, DH)
            probs[(s, h)] = _probabilities(queries.pop((s, h)), keys)

        def values(s, h):
            heads[(s, h)] = _weighted_values(probs.pop((s, h)), lambda b: v_v[s][b, h])
            i = h // TB
            ready = lambda m: all((s, m * TB + t) in heads for t in range(TB))
            if not ready(i):
                return
            a1 = lambda m: jnp.concatenate([heads[(s, m * TB + t)][0] for t in range(TB)], axis=1)
            a2 = lambda m: jnp.concatenate([heads[(s, m * TB + t)][1] for t in range(TB)], axis=1)
            made = _left_single(a1, a2, i)
            for m in range(NB):
                if m != i and ready(m):
                    made.update(_left_pair(a1, a2, min(i, m), max(i, m)))
            for prod, value in made.items():
                o_left[(s, prod)] = value

        for n, op in enumerate(ops):
            for gi in wait_at.get(n, []):
                for copy in copies(gi, None):
                    copy.wait()
            for u in start_at.get(n, []):
                for copy in copies(u % ng, u // ng, 1 - blk):
                    copy.start()
                if u < ng:
                    for copy in copies(u, 1, blk):
                        copy.start()
            if op[0] == "S":
                scores(op[1], op[2])
            elif op[0] == "V":
                values(op[1], op[2])
            else:
                product(*op)
            while results:
                tile, half, value = results.pop(0)
                rows = pl.ds(half * MH, MH)
                o_v[blk, tile, rows] = value.astype(BF16)
                cols = pl.ds(pl.multiple_of(blk * D + tile * 128, 128), 128)
                pltpu.make_async_copy(o_v.at[blk, tile, rows], out.at[rows, cols], out_sem).start()
        return trips + 1

    for u in ahead:
        for copy in copies(u, 0):
            copy.start()
    trips = lax.fori_loop(0, 2, attention_block, 0)
    for u in ahead:
        next(copies(u, 1, 2 - trips)).wait()
    pltpu.make_async_copy(o_v, o_v, out_sem).wait()


def _kernel(*refs):
    pl.run_scoped(lambda in_sem, out_sem: _both_blocks(*refs, in_sem, out_sem),
                  pltpu.SemaphoreType.DMA((_NSEM,)), pltpu.SemaphoreType.DMA(()))


@jax.jit
def pallas_concat_heads__mha_block_cached__mha_block_cached__near_ridge_kernel(
    A_x: jax.Array,
    A_k_cache: jax.Array,
    A_v_cache: jax.Array,
    A_wq: jax.Array,
    A_wo: jax.Array,
    B_x: jax.Array,
    B_k_cache: jax.Array,
    B_v_cache: jax.Array,
    B_wq: jax.Array,
    B_wo: jax.Array,
):
    in_hbm = pl.BlockSpec(memory_space=pl.ANY)
    out = pl.pallas_call(
        _kernel,
        out_shape=jax.ShapeDtypeStruct((M, 2 * D), BF16),
        in_specs=[in_hbm] * 10,
        out_specs=in_hbm,
        scratch_shapes=[
            pltpu.VMEM((B, SQ, D), BF16),
            [pltpu.VMEM((B, G, SK, DH), BF16) for _ in range(NS)],
            [pltpu.VMEM((B, G, SK, DH), BF16) for _ in range(NS)],
            [pltpu.VMEM((G, D, 128), BF16) for _ in range(NS)],
            [pltpu.VMEM((D // 128, G * DH, 128), BF16) for _ in range(NS)],
            pltpu.VMEM((2, D // 128, M, 128), BF16),
            pltpu.VMEM((8, 128), F32),
        ],
        compiler_params=pltpu.CompilerParams(
            vmem_limit_bytes=100 * 1024 * 1024,
            disable_bounds_checks=True,
            flags={"XLA_TPU_RESCHEDULE_DMA_DONES": True},
        ),
    )(A_x, A_k_cache, A_v_cache, A_wq, A_wo, B_x, B_k_cache, B_v_cache, B_wq, B_wo)
    return out.reshape(B, SQ, 2 * D)
```
